```python
import os as _os
_os.environ.setdefault("JAX_PLATFORMS", "cpu")
import jax
import jax.numpy as jnp

def _softmax(x, axis=-1):
    return jax.nn.softmax(x, axis=axis)
def _gelu(x):
    return jax.nn.gelu(x, approximate=True)
def _silu(x):
    return jax.nn.silu(x)
def _sigmoid(x):
    return jax.nn.sigmoid(x)
def _layernorm(x, axis=-1, eps=1e-5):
    m = jnp.mean(x, axis=axis, keepdims=True)
    v = jnp.var(x, axis=axis, keepdims=True)
    return (x - m) / jnp.sqrt(v + eps)
def _scatter_add(tgt, idx, src, axis=0):
    return tgt.at[idx].add(src)
def _segment_sum(src, seg, n):
    return jax.ops.segment_sum(src, seg, n)
class _Rng:
    def __init__(self, key):
        self._k = key
    def _next(self):
        self._k, sub = jax.random.split(self._k)
        return sub
    def normal(self, shape):
        return jax.random.normal(self._next(), shape, dtype=jnp.bfloat16)
    def randint(self, lo, hi, shape):
        return jax.random.randint(self._next(), shape, lo, hi, dtype=jnp.int32)
    def uniform(self, shape, lo=0.0, hi=1.0):
        return jax.random.uniform(self._next(), shape, jnp.bfloat16, lo, hi)
    def permutation(self, n):
        return jax.random.permutation(self._next(), n)


kernel_name = 'interleave_layers__spectral_gfnet__dense_activation_gelu__prompt'

def setup_inputs():
    _rng = _Rng(jax.random.key(int.from_bytes(__import__("os").urandom(4), "little")))
    _w = (lambda a: (lambda t: t.astype(jnp.bfloat16) if jnp.issubdtype(t.dtype, jnp.floating) else t)(jnp.asarray(a)))
    def _A_setup():
        B, S, D = 1, 2048, 640
        Df = D // 2 + 1
        return {
            "x": _w((lambda *s: _rng.normal(s) * 0.05)(B, S, D)),
            "w_r": _w((lambda *s: _rng.normal(s) * 0.2)(S, Df) * 0.02),
            "w_i": _w((lambda *s: _rng.normal(s) * 0.2)(S, Df) * 0.02),
        }
    _A_in = _A_setup()

    def _B_setup():
        B, S, D, F = 1, 2048, 640, 1728
        return {
            "x": _w((lambda *s: _rng.normal(s) * 0.05)(B, S, D)),
            "w1": _w((lambda *s: _rng.normal(s) * 0.1)(D, F) * (D ** -0.5)),
            "b1": _w((lambda *s: _rng.normal(s) * 0.1)(F) * 0.01),
            "w2": _w((lambda *s: _rng.normal(s) * 0.1)(F, D) * (F ** -0.5)),
            "b2": _w((lambda *s: _rng.normal(s) * 0.1)(D) * 0.01),
        }
    _B_in = _B_setup()

    return {
        "A_x": _A_in["x"],
        "A_w_r": _A_in["w_r"],
        "A_w_i": _A_in["w_i"],
        "B_x": _B_in["x"],
        "B_w1": _B_in["w1"],
        "B_b1": _B_in["b1"],
        "B_w2": _B_in["w2"],
        "B_b2": _B_in["b2"],
    }

def reference(A_x, A_w_r, A_w_i, B_x, B_w1, B_b1, B_w2, B_b2):
    def _A_ref(x, w_r, w_i):
        B, S, D = x.shape
        X = (lambda x, axes=(-2,-1): jnp.fft.rfft2(x.astype(jnp.float32), axes=axes))(x, axes=(-2, -1))
        W = w_r + 1j * w_i
        X = X * W
        y = (lambda x, s, axes=(-2,-1): jnp.fft.irfft2(x, s=s, axes=axes).astype(jnp.bfloat16))(X, (S, D), axes=(-2, -1))
        return y

    def _B_ref(x, w1, b1, w2, b2):
        h = jnp.einsum("bsd,df->bsf", x, w1) + b1
        h = _gelu(h)
        return jnp.einsum("bsf,fd->bsd", h, w2) + b2

    x = A_x
    x = x + _A_ref(_layernorm(x, axis=-1), A_w_r, A_w_i)
    x = x + _B_ref(_layernorm(x, axis=-1), B_w1, B_b1, B_w2, B_b2)
    x = x + _A_ref(_layernorm(x, axis=-1), A_w_r, A_w_i)
    x = x + _B_ref(_layernorm(x, axis=-1), B_w1, B_b1, B_w2, B_b2)
    return x
```

```python
import math

import numpy as np
import jax
import jax.numpy as jnp
import jax.experimental.pallas as pl
import jax.experimental.pallas.tpu as pltpu

S = 2048
D = 640
DF = D // 2 + 1
KP = 384
F = 1728
N1 = 16
N2 = S // N1
TM = 512


def _tables():
    d = np.arange(D)[:, None].astype(np.float64)
    k = np.arange(DF)[None, :].astype(np.float64)
    ang = 2.0 * np.pi * ((d * k) % D) / D
    fd = np.zeros((D, 2 * KP), np.float64)
    fd[:, :DF] = np.cos(ang)
    fd[:, KP:KP + DF] = -np.sin(ang)
    c = np.full((DF,), 2.0)
    c[0] = 1.0
    c[DF - 1] = 1.0
    c = c / (S * D)
    fi = np.zeros((2 * KP, D), np.float64)
    fi[:DF, :] = (np.cos(ang) * c[None, :]).T
    fi[KP:KP + DF, :] = (-np.sin(ang) * c[None, :]).T
    g = np.zeros((N1, 2 * N2, 2 * N2), np.float64)
    gi = np.zeros((N1, 2 * N2, 2 * N2), np.float64)
    kk = np.arange(N2)[:, None].astype(np.float64)
    for j in range(N1):
        ss = (j + N1 * np.arange(N2))[None, :].astype(np.float64)
        a = 2.0 * np.pi * ((kk * ss) % S) / S
        gr, gim = np.cos(a), -np.sin(a)
        g[j, :N2, :N2] = gr
        g[j, :N2, N2:] = -gim
        g[j, N2:, :N2] = gim
        g[j, N2:, N2:] = gr
        hr, him = np.cos(a).T, np.sin(a).T
        gi[j, :N2, :N2] = hr
        gi[j, :N2, N2:] = -him
        gi[j, N2:, :N2] = him
        gi[j, N2:, N2:] = hr
    return fd, fi, g, gi


_FD, _FI, _G, _GI = _tables()


def _cmul_const(re, im, c, s):
    if abs(s) < 1e-12:
        if abs(c - 1.0) < 1e-12:
            return re, im
        if abs(c + 1.0) < 1e-12:
            return -re, -im
    if abs(c) < 1e-12:
        if abs(s - 1.0) < 1e-12:
            return -im, re
        if abs(s + 1.0) < 1e-12:
            return im, -re
    if abs(abs(c) - abs(s)) < 1e-12:
        a = abs(c)
        sc = 1.0 if c > 0 else -1.0
        ss = 1.0 if s > 0 else -1.0
        r = (re - im) if sc == ss else (re + im)
        r = r * (a * sc)
        i = (re + im) if sc == ss else (im - re)
        i = i * (a * sc)
        return r, i
    return re * c - im * s, re * s + im * c


def _fft_list(xs, sign):
    n = len(xs)
    if n == 1:
        return xs
    ev = _fft_list(xs[0::2], sign)
    od = _fft_list(xs[1::2], sign)
    out = [None] * n
    for k in range(n // 2):
        ang = 2.0 * math.pi * k / n
        tr, ti = _cmul_const(od[k][0], od[k][1], math.cos(ang), sign * math.sin(ang))
        out[k] = (ev[k][0] + tr, ev[k][1] + ti)
        out[k + n // 2] = (ev[k][0] - tr, ev[k][1] - ti)
    return out


def _bf(x):
    return x.astype(jnp.bfloat16).astype(jnp.float32)


def _layernorm_bf16(x):
    m = jnp.mean(x, axis=-1, keepdims=True)
    xc = x - m
    v = jnp.mean(xc * xc, axis=-1, keepdims=True)
    dd = _bf(x - _bf(m))
    sd = _bf(jnp.sqrt(_bf(_bf(v) + 1e-5)))
    return (dd / sd).astype(jnp.bfloat16)


def _gelu(h):
    c = math.sqrt(2.0 / math.pi)
    return 0.5 * h * (1.0 + jnp.tanh(c * (h + 0.044715 * (h * h * h))))


GB = 8


def _kernel(x_hbm, wr_hbm, wi_hbm, w1t_hbm, b1_ref, w2_hbm, b2_ref,
            fd_hbm, fi_hbm, g_hbm, gi_hbm, o_ref,
            xb_ref, wrb_ref, wib_ref, w1t_ref, w2_ref, fd_ref, fi_ref, g_ref, gi_ref,
            xs_ref, wr_ref, wi_ref, z_ref, t3_ref, sems):
    copies = [
        pltpu.make_async_copy(x_hbm, xb_ref, sems.at[0]),
        pltpu.make_async_copy(fd_hbm, fd_ref, sems.at[1]),
        pltpu.make_async_copy(g_hbm, g_ref, sems.at[2]),
        pltpu.make_async_copy(wr_hbm, wrb_ref, sems.at[3]),
        pltpu.make_async_copy(wi_hbm, wib_ref, sems.at[4]),
        pltpu.make_async_copy(gi_hbm, gi_ref, sems.at[5]),
        pltpu.make_async_copy(fi_hbm, fi_ref, sems.at[6]),
        pltpu.make_async_copy(w1t_hbm, w1t_ref, sems.at[7]),
        pltpu.make_async_copy(w2_hbm, w2_ref, sems.at[8]),
    ]
    for cp in copies:
        cp.start()
    copies[0].wait()
    for lb in range(D // 128):
        t3_ref[lb] = xb_ref[:, lb * 128:(lb + 1) * 128].astype(jnp.float32)
    for j in range(N1):
        for lb in range(D // 128):
            xs_ref[j * N2:(j + 1) * N2, lb * 128:(lb + 1) * 128] = (
                t3_ref[lb, pl.ds(j, N2, stride=N1), :])
    copies[1].wait()

    def spectral_layer(first):
        def fwd(c, carry):
            r0 = pl.multiple_of(c * (GB * N2), GB * N2)
            xn = _layernorm_bf16(xs_ref[pl.ds(r0, GB * N2), :])
            a = jnp.dot(xn, fd_ref[...], preferred_element_type=jnp.float32)
            a = a.astype(jnp.bfloat16)
            for q in range(GB):
                j = c * GB + q
                aj = jnp.concatenate(
                    [a[q * N2:(q + 1) * N2, :KP], a[q * N2:(q + 1) * N2, KP:]], axis=0)
                z_ref[j] = jnp.dot(g_ref[j], aj, preferred_element_type=jnp.float32)
            return carry
        if first:
            copies[2].wait()
        lax_fori(0, N1 // GB, fwd, "fwd")

        if first:
            copies[3].wait()
            copies[4].wait()

            def wtr(b, carry):
                c0 = pl.multiple_of(b * N2, N2)
                for src, dst in ((wrb_ref, wr_ref), (wib_ref, wi_ref)):
                    for t in range(KP // 128):
                        lo, hi = t * 128, min((t + 1) * 128, DF)
                        tile = src[lo:hi, pl.ds(c0, N2)].astype(jnp.float32)
                        if hi - lo < 128:
                            tile = jnp.concatenate(
                                [tile, jnp.zeros((128 - (hi - lo), N2), jnp.float32)], axis=0)
                        dst[pl.ds(c0, N2), t * 128:(t + 1) * 128] = tile.T
                return carry
            lax_fori(0, N1, wtr, "wtr")

        def mid(t, carry):
            r0 = pl.multiple_of((t // 3) * 8, 8)
            l0 = pl.multiple_of((t % 3) * 128, 128)
            xs = []
            for b in range(N1):
                re = z_ref[b, pl.ds(r0, 8), pl.ds(l0, 128)]
                im = z_ref[b, pl.ds(N2 + r0, 8), pl.ds(l0, 128)]
                xs.append((re, im))
            ys = _fft_list(xs, -1)
            us = []
            for b in range(N1):
                wr = wr_ref[pl.ds(b * N2 + r0, 8), pl.ds(l0, 128)]
                wi = wi_ref[pl.ds(b * N2 + r0, 8), pl.ds(l0, 128)]
                yr, yi = ys[b]
                us.append((yr * wr - yi * wi, yr * wi + yi * wr))
            vs = _fft_list(us, +1)
            for b in range(N1):
                z_ref[b, pl.ds(r0, 8), pl.ds(l0, 128)] = vs[b][0]
                z_ref[b, pl.ds(N2 + r0, 8), pl.ds(l0, 128)] = vs[b][1]
            return carry
        lax_fori(0, (N2 // 8) * 3, mid, "mid", unroll=2)

        if first:
            copies[5].wait()
            copies[6].wait()

        def inv(c, carry):
            vs = []
            for q in range(GB):
                j = c * GB + q
                v = jnp.dot(gi_ref[j], z_ref[j].astype(jnp.bfloat16),
                            preferred_element_type=jnp.float32).astype(jnp.bfloat16)
                vs.append(jnp.concatenate([v[:N2], v[N2:]], axis=1))
            v = jnp.concatenate(vs, axis=0)
            y = jnp.dot(v, fi_ref[...], preferred_element_type=jnp.float32)
            r0 = pl.multiple_of(c * (GB * N2), GB * N2)
            rows = pl.ds(r0, GB * N2)
            xs_ref[rows, :] = _bf(xs_ref[rows, :] + _bf(y))
            return carry
        lax_fori(0, N1 // GB, inv, "inv")

    def mlp_layer(first):
        if first:
            copies[7].wait()
            copies[8].wait()
        b1 = b1_ref[...].astype(jnp.float32)
        b2 = b2_ref[...].astype(jnp.float32)

        def chunk(c, carry):
            r0 = pl.multiple_of(c * TM, TM)
            x = xs_ref[pl.ds(r0, TM), :]
            xn = _layernorm_bf16(x)
            h = jax.lax.dot_general(xn, w1t_ref[...], (((1,), (1,)), ((), ())),
                                    preferred_element_type=jnp.float32)
            h = _bf(_bf(h) + b1)
            h = _gelu(h).astype(jnp.bfloat16)
            y = _bf(jnp.dot(h, w2_ref[...], preferred_element_type=jnp.float32))
            y = _bf(y + b2)
            xs_ref[pl.ds(r0, TM), :] = _bf(x + y)
            return carry
        lax_fori(0, S // TM, chunk, "chunk")

    spectral_layer(True)
    mlp_layer(True)
    spectral_layer(False)
    mlp_layer(False)
    for j in range(N1):
        for lb in range(D // 128):
            t3_ref[lb, pl.ds(j, N2, stride=N1), :] = (
                xs_ref[j * N2:(j + 1) * N2, lb * 128:(lb + 1) * 128])
    for lb in range(D // 128):
        o_ref[:, lb * 128:(lb + 1) * 128] = t3_ref[lb].astype(jnp.bfloat16)


def lax_fori(lo, hi, body, name, unroll=1):
    with jax.named_scope(name):
        jax.lax.fori_loop(lo, hi, body, 0, unroll=unroll)


@jax.jit
def pallas_interleave_layers__spectral_gfnet__dense_activation_gelu__prompt_kernel(
    A_x: jax.Array,
    A_w_r: jax.Array,
    A_w_i: jax.Array,
    B_x: jax.Array,
    B_w1: jax.Array,
    B_b1: jax.Array,
    B_w2: jax.Array,
    B_b2: jax.Array,
):
    x = A_x.reshape(S, D)
    w1t = B_w1.T
    b1 = B_b1.reshape(1, F)
    b2 = B_b2.reshape(1, D)
    fd = jnp.asarray(_FD, jnp.bfloat16)
    fi = jnp.asarray(_FI, jnp.bfloat16)
    g = jnp.asarray(_G, jnp.bfloat16)
    gi = jnp.asarray(_GI, jnp.bfloat16)

    hbm = pl.BlockSpec(memory_space=pl.ANY)
    vmem = pl.BlockSpec(memory_space=pltpu.VMEM)
    out = pl.pallas_call(
        _kernel,
        out_shape=jax.ShapeDtypeStruct((S, D), jnp.bfloat16),
        in_specs=[hbm, hbm, hbm, hbm, vmem, hbm, vmem, hbm, hbm, hbm, hbm],
        out_specs=vmem,
        scratch_shapes=[
            pltpu.VMEM((S, D), jnp.bfloat16),
            pltpu.VMEM((DF, S), jnp.bfloat16),
            pltpu.VMEM((DF, S), jnp.bfloat16),
            pltpu.VMEM((F, D), jnp.bfloat16),
            pltpu.VMEM((F, D), jnp.bfloat16),
            pltpu.VMEM((D, 2 * KP), jnp.bfloat16),
            pltpu.VMEM((2 * KP, D), jnp.bfloat16),
            pltpu.VMEM((N1, 2 * N2, 2 * N2), jnp.bfloat16),
            pltpu.VMEM((N1, 2 * N2, 2 * N2), jnp.bfloat16),
            pltpu.VMEM((S, D), jnp.float32),
            pltpu.VMEM((S, KP), jnp.float32),
            pltpu.VMEM((S, KP), jnp.float32),
            pltpu.VMEM((N1, 2 * N2, KP), jnp.float32),
            pltpu.VMEM((D // 128, S, 128), jnp.float32),
            pltpu.SemaphoreType.DMA((9,)),
        ],
        compiler_params=pltpu.CompilerParams(
            vmem_limit_bytes=100 * 1024 * 1024,
        ),
    )(x, A_w_r.T, A_w_i.T, w1t, b1, B_w2, b2, fd, fi, g, gi)
    return out.reshape(1, S, D)
```
